```python
import os as _os
_os.environ.setdefault("JAX_PLATFORMS", "cpu")
import jax
import jax.numpy as jnp

def _softmax(x, axis=-1):
    return jax.nn.softmax(x, axis=axis)
def _gelu(x):
    return jax.nn.gelu(x, approximate=True)
def _silu(x):
    return jax.nn.silu(x)
def _sigmoid(x):
    return jax.nn.sigmoid(x)
def _layernorm(x, axis=-1, eps=1e-5):
    m = jnp.mean(x, axis=axis, keepdims=True)
    v = jnp.var(x, axis=axis, keepdims=True)
    return (x - m) / jnp.sqrt(v + eps)
def _scatter_add(tgt, idx, src, axis=0):
    return tgt.at[idx].add(src)
def _segment_sum(src, seg, n):
    return jax.ops.segment_sum(src, seg, n)
class _Rng:
    def __init__(self, key):
        self._k = key
    def _next(self):
        self._k, sub = jax.random.split(self._k)
        return sub
    def normal(self, shape):
        return jax.random.normal(self._next(), shape, dtype=jnp.bfloat16)
    def randint(self, lo, hi, shape):
        return jax.random.randint(self._next(), shape, lo, hi, dtype=jnp.int32)
    def uniform(self, shape, lo=0.0, hi=1.0):
        return jax.random.uniform(self._next(), shape, jnp.bfloat16, lo, hi)
    def permutation(self, n):
        return jax.random.permutation(self._next(), n)


kernel_name = 'recurrent_scan__grouped_kv_mqa__mixer_s_mlp__prompt'

def setup_inputs():
    _rng = _Rng(jax.random.key(int.from_bytes(__import__("os").urandom(4), "little")))
    _w = (lambda a: (lambda t: t.astype(jnp.bfloat16) if jnp.issubdtype(t.dtype, jnp.floating) else t)(jnp.asarray(a)))
    def _A_setup():
        B, S, D, H = 1, 2048, 512, 32
        Dh = D // H
        return {
            "x": _w((lambda *s: _rng.normal(s) * 0.05)(B, S, D)),
            "wq": _w((lambda *s: _rng.normal(s) * 0.05)(D, H * Dh)),
            "wk": _w((lambda *s: _rng.normal(s) * 0.05)(D, Dh)),
            "wv": _w((lambda *s: _rng.normal(s) * 0.05)(D, Dh)),
            "wo": _w((lambda *s: _rng.normal(s) * 0.05)(H * Dh, D)),
        }
    _A_in = _A_setup()

    def _B_setup():
        B, S, D, F = 1, 2048, 512, 1792
        return {
            "x":  _w((lambda *s: _rng.normal(s) * 0.05)(B, S, D)),
            "w1": _w((lambda *s: _rng.normal(s) * 0.8)(D, D) * (D ** -0.5)),
            "w2": _w((lambda *s: _rng.normal(s) * 0.8)(D, D) * (D ** -0.5)),
            "w3": _w((lambda *s: _rng.normal(s) * 0.8)(D, F) * (D ** -0.5)),
            "w4": _w((lambda *s: _rng.normal(s) * 0.8)(F, D) * (F ** -0.5)),
        }
    _B_in = _B_setup()

    return {
        "A_x": _A_in["x"],
        "A_wq": _A_in["wq"],
        "A_wk": _A_in["wk"],
        "A_wv": _A_in["wv"],
        "A_wo": _A_in["wo"],
        "B_x": _B_in["x"],
        "B_w1": _B_in["w1"],
        "B_w2": _B_in["w2"],
        "B_w3": _B_in["w3"],
        "B_w4": _B_in["w4"],
    }

def reference(A_x, A_wq, A_wk, A_wv, A_wo, B_x, B_w1, B_w2, B_w3, B_w4):
    def _A_ref(x, wq, wk, wv, wo):
        B, S, D = x.shape
        H = 32
        Dh = D // H
        q = (lambda x, *d: x.transpose(*d))((x @ wq).reshape(B, S, H, Dh), 0, 2, 1, 3)
        k = x @ wk
        v = x @ wv
        scores = jnp.einsum("bhqd,bkd->bhqk", q, k) * (Dh ** -0.5)
        p = _softmax(scores, axis=-1)
        o = jnp.einsum("bhqk,bkd->bhqd", p, v)
        return (lambda x, *d: x.transpose(*d))(o, 0, 2, 1, 3).reshape(B, S, H * Dh) @ wo

    def _B_ref(x, w1, w2, w3, w4):
        B, S, D = x.shape
        h = _gelu(_layernorm(x, axis=-1) @ w1)
        c = D // 4
        g0 = jnp.pad(h[:, :, 0*c:1*c], ((0, 0), (1, 0), (0, 0)))[:, :S, :]
        g1 = jnp.pad(h[:, :, 1*c:2*c], ((0, 0), (0, 1), (0, 0)))[:, 1:, :]
        g2 = jnp.pad(h[:, :, 2*c:3*c], ((0, 0), (2, 0), (0, 0)))[:, :S, :]
        g3 = jnp.pad(h[:, :, 3*c:   ], ((0, 0), (0, 2), (0, 0)))[:, 2:, :]
        hs = jnp.concatenate([g0, g1, g2, g3], axis=-1) @ w2
        x1 = x + hs
        h2 = _gelu(_layernorm(x1, axis=-1) @ w3) @ w4
        return x1 + h2

    x = A_x
    xn = _layernorm(x, axis=-1)
    s = _A_ref(xn, A_wq, A_wk, A_wv, A_wo)
    g = _silu(_B_ref(xn, B_w1, B_w2, B_w3, B_w4))
    return x + s * g
```

```python
import math

import jax
import jax.numpy as jnp
from jax import lax
import jax.experimental.pallas as pl
import jax.experimental.pallas.tpu as pltpu

S, D, H, DH, F = 2048, 512, 32, 16, 1792
RB = 512
QB = 512
CH = 128
NQ = S // QB
NITEM = H * NQ
PAD = 8
BF = jnp.bfloat16
F32 = jnp.float32
QSCALE = (DH ** -0.5) * math.log2(math.e)
NT = (((1,), (1,)), ((), ()))
TN = (((0,), (0,)), ((), ()))
UNROLL = 1


def _ln(x):
    m = jnp.mean(x, axis=-1, keepdims=True)
    c = x - m
    v = jnp.mean(c * c, axis=-1, keepdims=True)
    return c * lax.rsqrt(v + 1e-5)


def _gelu(x):
    c0 = math.sqrt(2.0 / math.pi)
    u = x * (c0 + (c0 * 0.044715) * (x * x))
    hx = 0.5 * x
    return hx + hx * jnp.tanh(u)


def _kernel(x_hbm, wq_hbm, wkT_hbm, wvT_hbm, wo_hbm, w1_hbm, w2_hbm, w3_hbm, w4_hbm,
            out_hbm,
            x_ref, wq_ref, wkT_ref, wvT_ref, wo_ref, w1_ref, w2_ref, w3_ref, w4_ref,
            wqT_ref, xn_ref, ln2_ref, qT_ref, k_ref, vT_ref, s_ref, oT_ref, h_ref, out_ref,
            xsem, wsem, osem):
    nb = S // RB

    def x_copy(r):
        rows = pl.ds(pl.multiple_of(r * RB, RB), RB)
        return pltpu.make_async_copy(x_hbm.at[rows], x_ref.at[rows], xsem.at[r])

    def o_copy(r):
        rows = pl.ds(pl.multiple_of(r * RB, RB), RB)
        return pltpu.make_async_copy(out_ref.at[rows], out_hbm.at[rows], osem.at[r])

    pairs = [(wq_hbm, wq_ref), (wkT_hbm, wkT_ref), (wvT_hbm, wvT_ref), (w1_hbm, w1_ref),
             (wo_hbm, wo_ref), (w2_hbm, w2_ref), (w3_hbm, w3_ref), (w4_hbm, w4_ref)]
    wc = [pltpu.make_async_copy(a, b, wsem.at[i]) for i, (a, b) in enumerate(pairs)]
    wc[0].start()
    x_copy(0).start()
    wc[1].start()
    wc[2].start()
    for r in range(1, nb):
        x_copy(r).start()
    for c in wc[3:]:
        c.start()

    wc[0].wait()
    wqT_ref[...] = wq_ref[...].astype(F32).T.astype(BF)
    wc[1].wait()
    wc[2].wait()

    def p0(r, carry):
        x_copy(r).wait()
        rows = pl.ds(pl.multiple_of(r * RB, RB), RB)
        xn = _ln(x_ref[rows, :].astype(F32)).astype(BF)
        xn_ref[rows, :] = xn
        ln2_ref[rows, :] = _ln(xn.astype(F32)).astype(BF)
        qT = lax.dot_general(wqT_ref[...], xn, NT, preferred_element_type=F32)
        qT_ref[r] = (qT * QSCALE).astype(BF).reshape(H, DH, RB)
        k_ref[rows, :] = lax.dot_general(xn, wkT_ref[...], NT, preferred_element_type=F32).astype(BF)
        vT_ref[r] = lax.dot_general(wvT_ref[...], xn, NT, preferred_element_type=F32).astype(BF)
        return carry

    lax.fori_loop(0, nb, p0, 0)

    def qk(j, qT):
        sn = jnp.dot(k_ref[j * CH:(j + 1) * CH, :], qT, preferred_element_type=F32)
        return sn, sn.reshape(CH // 8, 8, QB).max(0)

    def pv(j, m):
        s = s_ref[j * CH:(j + 1) * CH, :]
        p = jnp.exp2(s.reshape(CH // 8, 8, QB) - m[None])
        b, c = divmod(j * CH, RB)
        o = jnp.dot(vT_ref[b, :, c:c + CH], p.reshape(CH, QB).astype(BF), preferred_element_type=F32)
        return o, p.sum(0)

    def fin_max(mx):
        return jnp.broadcast_to(jnp.max(mx, axis=0, keepdims=True), (8, QB))

    def step(i, m, do_pv, do_qk):
        mx = l = o = None
        if do_qk:
            n = i + 1
            qT = qT_ref[n // H, n % H]
        for j in range(S // CH):
            if do_qk:
                sn, mj = qk(j, qT)
                mx = mj if mx is None else jnp.maximum(mx, mj)
            if do_pv:
                oj, lj = pv(j, m)
                l = lj if l is None else l + lj
                o = oj if o is None else o + oj
            if do_qk:
                s_ref[j * CH:(j + 1) * CH, :] = sn
        if do_pv:
            lt = jnp.sum(l, axis=0, keepdims=True)
            oT_ref[i // H, i % H] = (o * (1.0 / lt)).astype(BF)
        return fin_max(mx) if do_qk else None

    m0 = step(-1, None, False, True)
    ml = lax.fori_loop(0, NITEM - 1, lambda i, m: step(i, m, True, True), m0, unroll=UNROLL)
    step(NITEM - 1, ml, True, False)

    wc[3].wait()
    h_ref[:, 0:PAD, :] = jnp.zeros((4, PAD, 128), F32)
    h_ref[:, PAD + S:, :] = jnp.zeros((4, PAD, 128), F32)

    def p2(r, carry):
        r0 = pl.multiple_of(r * RB, RB)
        a = jnp.dot(ln2_ref[pl.ds(r0, RB), :], w1_ref[...], preferred_element_type=F32)
        h = _gelu(a)
        for g in range(4):
            h_ref[g, pl.ds(r0 + PAD, RB), :] = h[:, g * 128:(g + 1) * 128]
        return carry

    lax.fori_loop(0, nb, p2, 0)

    for c in wc[4:]:
        c.wait()

    def p3(r, carry):
        r0 = pl.multiple_of(r * RB, RB)
        rows = pl.ds(r0, RB)
        parts = []
        for g, sh in enumerate((1, -1, 2, -2)):
            parts.append(h_ref[g, pl.ds(r0 + (PAD - sh), RB), :].astype(BF))
        hs = jnp.dot(jnp.concatenate(parts, axis=-1), w2_ref[...], preferred_element_type=F32)
        x1 = xn_ref[rows, :].astype(F32) + hs
        a = jnp.dot(_ln(x1).astype(BF), w3_ref[...], preferred_element_type=F32)
        b = x1 + jnp.dot(_gelu(a).astype(BF), w4_ref[...], preferred_element_type=F32)
        hb = 0.5 * b
        gate = hb + hb * jnp.tanh(hb)
        sa = lax.dot_general(oT_ref[r].reshape(D, RB), wo_ref[...], TN, preferred_element_type=F32)
        out_ref[rows, :] = (x_ref[rows, :].astype(F32) + sa * gate).astype(BF)
        o_copy(r).start()
        return carry

    lax.fori_loop(0, nb, p3, 0)
    for r in range(nb):
        o_copy(r).wait()


@jax.jit
def pallas_recurrent_scan__grouped_kv_mqa__mixer_s_mlp__prompt_kernel(
    A_x: jax.Array,
    A_wq: jax.Array,
    A_wk: jax.Array,
    A_wv: jax.Array,
    A_wo: jax.Array,
    B_x: jax.Array,
    B_w1: jax.Array,
    B_w2: jax.Array,
    B_w3: jax.Array,
    B_w4: jax.Array,
):
    del B_x
    any_spec = pl.BlockSpec(memory_space=pl.ANY)
    vm = pltpu.VMEM
    out = pl.pallas_call(
        _kernel,
        out_shape=jax.ShapeDtypeStruct((S, D), BF),
        in_specs=[any_spec] * 9,
        out_specs=any_spec,
        scratch_shapes=[
            vm((S, D), BF), vm((D, D), BF), vm((DH, D), BF), vm((DH, D), BF), vm((D, D), BF),
            vm((D, D), BF), vm((D, D), BF), vm((D, F), BF), vm((F, D), BF),
            vm((D, D), BF), vm((S, D), BF), vm((S, D), BF), vm((NQ, H, DH, QB), BF),
            vm((S, DH), BF), vm((S // RB, DH, RB), BF), vm((S, QB), F32), vm((NQ, H, DH, QB), BF),
            vm((4, S + 2 * PAD, 128), F32), vm((S, D), BF),
            pltpu.SemaphoreType.DMA((S // RB,)), pltpu.SemaphoreType.DMA((8,)),
            pltpu.SemaphoreType.DMA((S // RB,)),
        ],
        compiler_params=pltpu.CompilerParams(vmem_limit_bytes=100 << 20),
        name="fused",
    )(A_x.reshape(S, D), A_wq, A_wk.T, A_wv.T, A_wo, B_w1, B_w2, B_w3, B_w4)
    return out.reshape(1, S, D)
```

```python
import math

import jax
import jax.numpy as jnp
from jax import lax
import jax.experimental.pallas as pl
import jax.experimental.pallas.tpu as pltpu

S, D, H, DH, F = 2048, 512, 32, 16, 1792
RB = 512
NB = S // RB
CH = 128
NV = 16
NM = CH - NV
NS = S // CH
NITEM = H * NB
LAG = 2
U = 8
TQ = 4
SL = 16
W4S = 64
W4K = 14
FLAGS = {"XLA_TPU_EVENLY_DISTRIBUTE_CRITICAL_NODES": True}
HALO = 16
SLABS = tuple((i * SL, SL) for i in range((RB + 2 * HALO) // SL))
L3 = ((0, 192), (192, 384), (384, 512))
BF = jnp.bfloat16
F32 = jnp.float32
QSCALE = (DH ** -0.5) * math.log2(math.e)
L_LO, L_HI = 2.0 ** -40, 2.0 ** 40
NT = (((1,), (1,)), ((), ()))


def _ln(x):
    m = jnp.sum(x, axis=-1, keepdims=True) * (1.0 / D)
    c = x - m
    v = jnp.sum(c * c, axis=-1, keepdims=True) * (1.0 / D)
    return c * lax.rsqrt(v + 1e-5)


def _gelu(x):
    c0 = math.sqrt(2.0 / math.pi)
    u = x * (c0 + (c0 * 0.044715) * (x * x))
    hx = 0.5 * x
    return hx + hx * jnp.tanh(u)


def _bf_round(x):
    return x.astype(BF).astype(F32)


def _kernel(x_hbm, wq_hbm, wkT_hbm, wvT_hbm, wo_hbm, w1_hbm, w2_hbm, w3_hbm, w4_hbm,
            out_hbm,
            x_ref, wq_ref, wo_ref, w1_ref, w2_ref, w3_ref, w4_ref,
            wT_ref, xn_ref, ln2_ref, qT_ref, qb_ref, kf_ref, k_ref, kb_ref, vT_ref, p_ref, o_ref, l_ref,
            h_ref, x1_ref, ln3_ref, a_ref, g_ref, out_ref, wsem, osem):
    def rows_of(r):
        return pl.ds(pl.multiple_of(r * RB, RB), RB)

    def o_copy(r, c):
        rows = pl.ds(pl.multiple_of(r * RB + c * 128, 128), 128)
        return pltpu.make_async_copy(out_ref.at[rows], out_hbm.at[rows], osem.at[r])

    n0 = RB + HALO
    pairs = [(x_hbm.at[pl.ds(0, n0)], x_ref.at[pl.ds(HALO, n0)]), (w1_hbm, w1_ref),
             (wq_hbm, wq_ref), (w2_hbm, w2_ref),
             (wkT_hbm, wT_ref.at[pl.ds(D, DH)]), (wvT_hbm, wT_ref.at[pl.ds(D + DH, DH)]),
             (w3_hbm, w3_ref), (w4_hbm, w4_ref),
             (x_hbm.at[pl.ds(n0, S - n0)], x_ref.at[pl.ds(HALO + n0, S - n0)]), (wo_hbm, wo_ref)]
    wc = [pltpu.make_async_copy(a, b, wsem.at[i]) for i, (a, b) in enumerate(pairs)]
    for n in (0, 2, 4, 5, 1, 3):
        wc[n].start()

    x_ref[0:HALO, :] = jnp.zeros((HALO, D), BF)
    x_ref[HALO + S:2 * HALO + S, :] = jnp.zeros((HALO, D), BF)
    p_ref[...] = jnp.zeros_like(p_ref)
    o_ref[0] = jnp.zeros((DH, RB), F32)

    def norms(r0, lo, n):
        xn = _ln(x_ref[pl.ds(r0 + lo, n), :].astype(F32)).astype(BF)
        xn_ref[lo:lo + n, :] = xn
        ln2_ref[lo:lo + n, :] = _ln(xn.astype(F32)).astype(BF)

    wc[0].wait()
    norms(0, 0, RB + 2 * HALO)
    wc[2].wait()
    wT_ref[0:D, :] = wq_ref[...].astype(F32).T.astype(BF)
    for c in wc[1:2] + wc[3:6]:
        c.wait()
    wc[6].start()
    wc[8].start()

    def pa(r, k2max):
        r0 = pl.multiple_of(r * RB, RB)

        hh = _gelu(jnp.dot(ln2_ref[...], w1_ref[...], preferred_element_type=F32))
        for g in range(4):
            h_ref[g] = hh[:, g * 128:(g + 1) * 128]
        parts = [h_ref[g, HALO - sh:HALO - sh + RB, :].astype(BF)
                 for g, sh in enumerate((1, -1, 2, -2))]
        hs = jnp.dot(jnp.concatenate(parts, axis=-1), w2_ref[...], preferred_element_type=F32)
        x1 = xn_ref[HALO:HALO + RB, :].astype(F32) + hs
        x1_ref[...] = x1
        for t in range(4):
            y = lax.dot_general(wT_ref[t * 128:(t + 1) * 128 + (2 * DH if t == 3 else 0), :],
                                xn_ref[HALO:HALO + RB, :], NT, preferred_element_type=F32)
            for h in range(8):
                qT_ref[r * H + t * 8 + h, 0:DH, :] = (y[h * DH:(h + 1) * DH] * QSCALE).astype(BF)
            if t < len(L3):
                lo, hi = L3[t]
                ln3_ref[lo:hi, :] = _ln(x1_ref[lo:hi, :]).astype(BF)
        kT = _bf_round(y[128:128 + DH])
        vT_ref[r] = pltpu.bitcast(y[128 + DH:].astype(BF), jnp.uint32)

        @pl.when(r == 0)
        def _():
            wc[7].start()
            wc[6].wait()
            wc[8].wait()

        a = jnp.dot(ln3_ref[...], w3_ref[...], preferred_element_type=F32)
        act = _gelu(a).astype(BF)
        a_ref[...] = act
        rn = pl.multiple_of(jnp.minimum(r + 1, NB - 1) * RB, RB)
        for sl, (lo, m) in enumerate(SLABS):
            grp, pos = divmod(sl * 3 * (RB // DH) // len(SLABS), RB // DH)
            x_ref[S + 2 * HALO:, 0:128] = act[pos * DH:(pos + 1) * DH, grp * 512:grp * 512 + 128]
            norms(rn, lo, m)

        @pl.when(r == 0)
        def _():
            wc[9].start()
            wc[7].wait()

        kf = jnp.concatenate([kT, jnp.zeros((128 - DH, RB), F32)], axis=0).T
        kf_ref[rows_of(r), :] = kf
        nsl = RB // W4S
        b = None
        for t in range(nsl):
            for kk in range(W4K):
                if b is not None:
                    qT_ref[NITEM, 0:DH, 0:128] = b[0:DH, 0:128].astype(BF)
                if kk == 0:
                    b = x1_ref[t * W4S:(t + 1) * W4S, :]
                fk = slice(kk * (F // W4K), (kk + 1) * (F // W4K))
                b = b + jnp.dot(a_ref[t * W4S:(t + 1) * W4S, fk], w4_ref[fk, :],
                                preferred_element_type=F32)
                n = t * W4K + kk
                for u in range(H * TQ):
                    if u * (nsl * W4K - 1) // (H * TQ) != n:
                        continue
                    h, part = divmod(u, TQ)
                    i = r * H + h
                    qf = qT_ref[i, 0:DH, :].astype(F32)
                    for d in range(part * DH // TQ, (part + 1) * DH // TQ):
                        qb_ref[i, d] = jnp.broadcast_to(qf[d:d + 1], (8, RB))
                    if part == 0:
                        qn = jnp.sqrt(jnp.sum(qf * qf, axis=0, keepdims=True))
                        qn = _bf_round(qn * (1.0 + 2.0 ** -6))
                        qT_ref[i, DH:, :] = jnp.broadcast_to(qn, (DH, RB)).astype(BF)
                        qb_ref[i, DH] = jnp.broadcast_to(qn, (8, RB))
                    if part == TQ - 1:
                        c, d0 = divmod(h, 8)
                        kv = kf_ref[pl.ds(r0 + c * CH + NM, NV), :]
                        for d in (2 * d0, 2 * d0 + 1):
                            kb_ref[r * (RB // CH) + c, d] = jnp.broadcast_to(
                                kv[:, d:d + 1], (NV, 128))
            hb = 0.5 * b
            g_ref[pl.ds(r0 + t * W4S, W4S), :] = hb + hb * jnp.tanh(hb)
        return jnp.maximum(k2max, jnp.sum(kT * kT, axis=0, keepdims=True))

    k2max = lax.fori_loop(0, NB, pa, jnp.zeros((1, RB), F32))
    kc = _bf_round(jnp.sqrt(jnp.max(k2max, axis=1, keepdims=True)) * (-(1.0 + 2.0 ** -6) / DH))
    kneg = jnp.broadcast_to(kc * DH, (8, RB))
    lane = lax.broadcasted_iota(jnp.int32, (CH, 128), 1)
    for j in range(NS):
        ka = jnp.where((lane >= DH) & (lane < 2 * DH), kc, kf_ref[j * CH:(j + 1) * CH, :])
        k_ref[j] = pltpu.bitcast(ka.astype(BF), jnp.uint32)

    def v_chunk(j):
        b, c = divmod(j * CH, RB)
        return pltpu.bitcast(vT_ref[b, :, c:c + CH], BF)

    def put_l(i, l):
        for c in range(RB // 128):
            l_ref[c, pl.ds(pl.multiple_of(i * 8, 8), 8), :] = l[:, c * 128:(c + 1) * 128]

    def attn(it, carry):
        ps = {t - LAG: p_ref[t] for t in range(LAG)}
        ls = {}
        acc_o = {-1: o_ref[it * U]}

        def scores(g):
            u, j = divmod(g, NS)
            i = it * U + u
            kk = pltpu.bitcast(k_ref[j, 0:NM // 2, :], BF)[:, :2 * DH]
            p_mxu = jnp.exp2(jnp.dot(kk, qT_ref[i], preferred_element_type=F32))
            acc = qb_ref[i, DH] * kneg
            if g >= 2:
                acc = acc + ls[g - 2] * 0.0
            acc = acc[None]
            for d in range(DH):
                kb = kb_ref[j, d]
                kb = jnp.concatenate([kb] * (RB // 128), axis=1).reshape(NV // 8, 8, RB)
                acc = acc + kb * qb_ref[i, d][None]
            p = jnp.concatenate([p_mxu, jnp.exp2(acc).reshape(NV, RB)], axis=0)
            lj = p.reshape(CH // 8, 8, RB).sum(0)
            ls[g] = lj if j == 0 else ls[g - 1] + lj
            if j == NS - 1:
                put_l(i, ls[g])
            ps[g] = p.astype(BF)

        def pv(g):
            u, j = divmod(g, NS)
            oj = jnp.dot(v_chunk(j), ps.pop(g), preferred_element_type=F32)
            acc_o[u] = oj + (acc_o[u - 1] * 0.0 if j == 0 else acc_o[u])
            if j == NS - 1 or g == U * NS - LAG - 1:
                o_ref[it * U + u + 1] = acc_o[u]

        for g in range(U * NS):
            scores(g)
            pv(g - LAG)
        for t in range(LAG):
            p_ref[t] = ps[U * NS - LAG + t]
        return carry

    lax.fori_loop(0, NITEM // U, attn, 0)
    o_last = o_ref[NITEM]
    for t in range(LAG):
        o_last = o_last + jnp.dot(v_chunk(NS - LAG + t), p_ref[t], preferred_element_type=F32)
    o_ref[NITEM] = o_last

    def attn_true_max(i, carry):
        q = qT_ref[i, 0:DH, :]

        def sc(j):
            return jnp.dot(pltpu.bitcast(k_ref[j], BF)[:, :DH], q, preferred_element_type=F32)

        m = lax.fori_loop(
            0, NS, lambda j, m: jnp.maximum(m, jnp.max(sc(j), axis=0, keepdims=True)),
            jnp.full((1, RB), -jnp.inf, F32))
        o = jnp.zeros((DH, RB), F32)
        l = jnp.zeros((8, RB), F32)
        for j in range(NS):
            p = jnp.exp2(sc(j) - m)
            l = l + p.reshape(CH // 8, 8, RB).sum(0)
            o = o + jnp.dot(v_chunk(j), p.astype(BF), preferred_element_type=F32)
        o_ref[i + 1] = o
        put_l(i, l)
        return carry

    wc[9].wait()

    def p2(r, bad):
        def normalized(c, bad):
            heads = []
            for h0 in range(0, H, 8):
                base = (r * H + h0) * 8
                lt = l_ref[c, pl.ds(base, 8, stride=8), :]
                for t in range(1, 8):
                    lt = lt + l_ref[c, pl.ds(base + t, 8, stride=8), :]
                bad = jnp.where((lt >= L_LO) & (lt <= L_HI), bad, 1.0)
                inv = 1.0 / lt
                for h in range(8):
                    o = o_ref[r * H + h0 + h + 1, :, c * 128:(c + 1) * 128]
                    heads.append((o * inv[h:h + 1]).astype(BF))
            return jnp.concatenate(heads, axis=0).T, bad

        nxt, bad = normalized(0, bad)
        for c in range(RB // 128):
            cur = nxt
            if c + 1 < RB // 128:
                nxt, bad = normalized(c + 1, bad)
            sa = jnp.dot(cur, wo_ref[...], preferred_element_type=F32)
            lo = pl.multiple_of(r * RB + c * 128, 128)
            x = x_ref[pl.ds(lo + HALO, 128), :].astype(F32)
            out_ref[pl.ds(lo, 128), :] = (x + sa * g_ref[pl.ds(lo, 128), :]).astype(BF)
            o_copy(r, c).start()
        return bad

    def finish():
        bad = lax.fori_loop(0, NB, p2, jnp.zeros((8, 128), F32))
        for r in range(NB):
            for c in range(RB // 128):
                o_copy(r, c).wait()
        return bad

    bad = jnp.maximum(jnp.max(finish()), jnp.max(jnp.where(o_last == o_last, 0.0, 1.0)))

    @pl.when(bad > 0.0)
    def _():
        lax.fori_loop(0, NITEM, attn_true_max, 0)
        finish()


@jax.jit
def pallas_recurrent_scan__grouped_kv_mqa__mixer_s_mlp__prompt_kernel(
    A_x: jax.Array,
    A_wq: jax.Array,
    A_wk: jax.Array,
    A_wv: jax.Array,
    A_wo: jax.Array,
    B_x: jax.Array,
    B_w1: jax.Array,
    B_w2: jax.Array,
    B_w3: jax.Array,
    B_w4: jax.Array,
):
    del B_x
    any_spec = pl.BlockSpec(memory_space=pl.ANY)
    vm = pltpu.VMEM
    out = pl.pallas_call(
        _kernel,
        out_shape=jax.ShapeDtypeStruct((S, D), BF),
        in_specs=[any_spec] * 9,
        out_specs=any_spec,
        scratch_shapes=[
            vm((S + 2 * HALO + DH, D), BF), vm((D, D), BF), vm((D, D), BF), vm((D, D), BF), vm((D, D), BF),
            vm((D, F), BF), vm((F, D), BF),
            vm((D + 2 * DH, D), BF), vm((RB + 2 * HALO, D), BF), vm((RB + 2 * HALO, D), BF),
            vm((NITEM + 1, 2 * DH, RB), BF), vm((NITEM, DH + 1, 8, RB), F32),
            vm((S, 128), F32), vm((NS, CH // 2, 128), jnp.uint32), vm((NS, DH, NV, 128), F32),
            vm((NB, DH // 2, RB), jnp.uint32), vm((LAG, CH, RB), BF),
            vm((NITEM + 1, DH, RB), F32), vm((RB // 128, NITEM * 8 + 8, 128), F32),
            vm((4, RB + 2 * HALO, 128), F32), vm((RB, D), F32), vm((RB, D), BF), vm((RB, F), BF),
            vm((S, D), F32), vm((S, D), BF),
            pltpu.SemaphoreType.DMA((10,)),
            pltpu.SemaphoreType.DMA((NB,)),
        ],
        compiler_params=pltpu.CompilerParams(vmem_limit_bytes=110 << 20, flags=FLAGS),
        name="fused",
    )(A_x.reshape(S, D), A_wq, A_wk.T, A_wv.T, A_wo, B_w1, B_w2, B_w3, B_w4)
    return out.reshape(1, S, D)
```
